```python
import jax
import jax.numpy as jnp

def _softmax(x, axis=-1):
    return jax.nn.softmax(x, axis=axis)
def _gelu(x):
    return jax.nn.gelu(x, approximate=True)
def _silu(x):
    return jax.nn.silu(x)
def _sigmoid(x):
    return jax.nn.sigmoid(x)
def _layernorm(x, axis=-1, eps=1e-5):
    m = jnp.mean(x, axis=axis, keepdims=True)
    v = jnp.var(x, axis=axis, keepdims=True)
    return (x - m) / jnp.sqrt(v + eps)
def _scatter_add(tgt, idx, src, axis=0):
    return tgt.at[idx].add(src)
def _segment_sum(src, seg, n):
    return jax.ops.segment_sum(src, seg, n)
class _Rng:
    def __init__(self, key):
        self._k = key
    def _next(self):
        self._k, sub = jax.random.split(self._k)
        return sub
    def normal(self, shape):
        return jax.random.normal(self._next(), shape, dtype=jnp.bfloat16)
    def randint(self, lo, hi, shape):
        return jax.random.randint(self._next(), shape, lo, hi, dtype=jnp.int32)
    def uniform(self, shape, lo=0.0, hi=1.0):
        return jax.random.uniform(self._next(), shape, jnp.bfloat16, lo, hi)
    def permutation(self, n):
        return jax.random.permutation(self._next(), n)


kernel_name = 'sequential_preLN__mha_block_cached__moe_arch_mod__decode'

def setup_inputs():
    _rng = _Rng(jax.random.key(int.from_bytes(__import__("os").urandom(4), "little")))
    _w = (lambda a: (lambda t: t.astype(jnp.bfloat16) if jnp.issubdtype(t.dtype, jnp.floating) else t)(jnp.asarray(a)))
    def _A_setup():
        B, Sq, D = 4, 1, 640
        H, Sk, Dh = 32, 8192, 192
        return {
            "x": _w((lambda *s: _rng.normal(s) * 0.05)(B, Sq, D)),
            "k_cache": _w((lambda *s: _rng.normal(s) * 0.05)(B, H, Sk, Dh)),
            "v_cache": _w((lambda *s: _rng.normal(s) * 0.05)(B, H, Sk, Dh)),
            "wq": _w((lambda *s: _rng.normal(s) * 0.05)(D, H * Dh) * (D ** -0.5)),
            "wo": _w((lambda *s: _rng.normal(s) * 0.05)(H * Dh, D) * ((H * Dh) ** -0.5)),
        }
    _A_in = _A_setup()

    def _B_setup():
        B, S, D, F, C = 4, 1, 640, 1536, 1
        return {
            "x": _w((lambda *s: _rng.normal(s) * 0.05)(B, S, D)),
            "w_r": _w((lambda *s: _rng.normal(s) * 0.05)(D)),
            "w_gate": _w((lambda *s: _rng.normal(s) * 0.05)(D, F)),
            "w_up": _w((lambda *s: _rng.normal(s) * 0.05)(D, F)),
            "w_down": _w((lambda *s: _rng.normal(s) * 0.05)(F, D)),
        }
    _B_in = _B_setup()

    return {
        "A_x": _A_in["x"],
        "A_k_cache": _A_in["k_cache"],
        "A_v_cache": _A_in["v_cache"],
        "A_wq": _A_in["wq"],
        "A_wo": _A_in["wo"],
        "B_x": _B_in["x"],
        "B_w_r": _B_in["w_r"],
        "B_w_gate": _B_in["w_gate"],
        "B_w_up": _B_in["w_up"],
        "B_w_down": _B_in["w_down"],
    }

def reference(A_x, A_k_cache, A_v_cache, A_wq, A_wo, B_x, B_w_r, B_w_gate, B_w_up, B_w_down):
    def _A_ref(x, k_cache, v_cache, wq, wo):
        B, Sq, D = x.shape
        H, Dh = 32, 192
        q = (lambda x, *d: x.transpose(*d))((x @ wq).reshape(B, Sq, H, Dh), 0, 2, 1, 3)
        scores = jnp.einsum("bhqd,bhkd->bhqk", q, k_cache) * (Dh ** -0.5)
        p = _softmax(scores, axis=-1)
        o = jnp.einsum("bhqk,bhkd->bhqd", p, v_cache)
        return (lambda x, *d: x.transpose(*d))(o, 0, 2, 1, 3).reshape(B, Sq, H * Dh) @ wo

    def _B_ref(x, w_r, w_gate, w_up, w_down):
        B, S, D = x.shape
        C = 1
        r = x @ w_r
        idx = jnp.argsort(-r, axis=-1)[:, :C]
        idx_e = jnp.repeat(idx.reshape(B, C, 1), D, axis=2)
        x_sel = jnp.take_along_axis(x, idx_e, axis=1)
        g = _silu(x_sel @ w_gate)
        u = x_sel @ w_up
        y = (g * u) @ w_down
        r_sel = _sigmoid(jnp.take_along_axis(r, idx, axis=1))
        y = y * r_sel.reshape(B, C, 1)
        b_off = (jnp.arange(B) * S).reshape(B, 1)
        flat_idx = (idx + b_off).reshape(B * C)
        zero = (x * 0.0).reshape(B * S, D)
        upd = _scatter_add(zero, flat_idx, y.reshape(B * C, D), axis=0)
        return x + upd.reshape(B, S, D)

    x = A_x
    h = x + _A_ref(_layernorm(x, axis=-1), A_k_cache, A_v_cache, A_wq, A_wo)
    h2 = h + _B_ref(_layernorm(h, axis=-1), B_w_r, B_w_gate, B_w_up, B_w_down)
    return h2
```

```python
import functools

import jax
import jax.numpy as jnp
from jax import lax
import jax.experimental.pallas as pl
import jax.experimental.pallas.tpu as pltpu

F32 = jnp.float32
BF16 = jnp.bfloat16

ROWS = 8
BLK = 1024
CH_R = 16
CH_C = 1024
NSLOT = 4
NT = (((1,), (1,)), ((), ()))


def _layernorm(x):
    m = jnp.mean(x, axis=-1, keepdims=True)
    xc = x - m
    v = jnp.mean(xc * xc, axis=-1, keepdims=True)
    return xc / jnp.sqrt(v + 1e-5)


def _kernel(x_hbm, k_hbm, v_hbm, wq_hbm, wo_hbm, wr_hbm, wg_hbm, wu_hbm, wd_hbm,
            o_ref,
            kv_buf, x_buf, wq_buf, wo_buf, wr_buf, wg_buf, wu_buf, wd_buf,
            q_buf, qbd_ref, m_ref, l_ref, acc_ref, attn_ref, kv_sem, w_sem,
            *, B, H, Dh, S, D, F):
    J = S // BLK
    NU = H * J
    scale = Dh ** -0.5

    def start_rows(src, dst, sem, rows):
        n = src.shape[0] // rows
        for i in range(n):
            sl = pl.ds(i * rows, rows)
            pltpu.make_async_copy(src.at[sl], dst.at[sl], sem).start(priority=i % 2)

    def wait_all(dst, sem):
        pltpu.make_async_copy(dst, dst, sem).wait()

    def start_unit(u, slot):
        h = u // J
        j = u % J
        for g in range(Dh // CH_R):
            for c in range(BLK // CH_C):
                col = pl.ds(pl.multiple_of(j * BLK + c * CH_C, CH_C), CH_C)
                for kv, src in enumerate((k_hbm, v_hbm)):
                    for b in range(B):
                        pltpu.make_async_copy(
                            src.at[b, h, pl.ds(g * CH_R, CH_R), col],
                            kv_buf.at[slot, kv, pl.ds(b * Dh + g * CH_R, CH_R),
                                      pl.ds(c * CH_C, CH_C)],
                            kv_sem.at[slot]).start(priority=b % 2)

    pltpu.make_async_copy(x_hbm, x_buf, w_sem.at[0]).start()
    start_rows(wq_hbm, wq_buf, w_sem.at[1], 16)
    pltpu.make_async_copy(wr_hbm, wr_buf, w_sem.at[2]).start()
    for s in range(NSLOT - 1):
        start_unit(s, s)
    start_rows(wo_hbm, wo_buf, w_sem.at[3], 32)

    wait_all(x_buf, w_sem.at[0])
    x = jnp.concatenate(
        [x_buf[...].astype(F32), jnp.zeros((ROWS - B, D), F32)], axis=0)
    xn = _layernorm(x).astype(BF16)
    wait_all(wq_buf, w_sem.at[1])
    q = jnp.dot(xn, wq_buf[...], preferred_element_type=F32)
    q = q.astype(BF16).astype(F32)
    for h in range(H):
        q_buf[h] = q[:, h * Dh:(h + 1) * Dh]
    attn_ref[...] = jnp.zeros_like(attn_ref)

    row_bd = lax.broadcasted_iota(jnp.int32, (ROWS, B * Dh), 0)
    col_bd = lax.broadcasted_iota(jnp.int32, (ROWS, B * Dh), 1)
    on_diag = (col_bd >= row_bd * Dh) & (col_bd < (row_bd + 1) * Dh)
    row_h = lax.broadcasted_iota(jnp.int32, (ROWS, Dh), 0)

    def compute_unit(u, slot):
        h = u // J
        j = u % J

        @pl.when(j == 0)
        def _():
            qh = q_buf[h]
            qbd = jnp.concatenate([qh] * B, axis=1)
            qbd_ref[...] = jnp.where(on_diag, qbd, 0.0)
            m_ref[...] = jnp.full_like(m_ref, -jnp.inf)
            l_ref[...] = jnp.zeros_like(l_ref)
            acc_ref[...] = jnp.zeros_like(acc_ref)

        s = jnp.dot(qbd_ref[...].astype(BF16), kv_buf[slot, 0],
                    preferred_element_type=F32) * scale
        m_old = m_ref[...]
        m_new = jnp.maximum(m_old, jnp.max(s, axis=-1, keepdims=True))
        alpha = jnp.exp(m_old - m_new)
        p = jnp.exp(s - m_new)
        l_ref[...] = alpha * l_ref[...] + jnp.sum(p, axis=-1, keepdims=True)
        m_ref[...] = m_new
        pv = lax.dot_general(p.astype(BF16), kv_buf[slot, 1], NT,
                             preferred_element_type=F32)
        acc_ref[...] = alpha * acc_ref[...] + pv

        @pl.when(j == J - 1)
        def _():
            @pl.when(h == 0)
            def _():
                wait_all(wo_buf, w_sem.at[3])

            acc = acc_ref[...]
            o = jnp.zeros((ROWS, Dh), F32)
            for b in range(B):
                o = jnp.where(row_h == b, acc[:, b * Dh:(b + 1) * Dh], o)
            o = (o / l_ref[...]).astype(BF16)
            wo_h = wo_buf[pl.ds(pl.multiple_of(h * Dh, Dh), Dh), :]
            attn_ref[...] += jnp.dot(o, wo_h, preferred_element_type=F32)

    def body(u, carry):
        slot = u % NSLOT
        wait_all(kv_buf.at[slot], kv_sem.at[slot])
        nxt = u + NSLOT - 1
        start_unit(nxt, nxt % NSLOT)
        compute_unit(u, slot)
        return carry

    lax.fori_loop(0, NU - NSLOT + 1, body, 0)

    start_rows(wg_hbm, wg_buf, w_sem.at[4], 16)
    start_rows(wu_hbm, wu_buf, w_sem.at[5], 16)
    start_rows(wd_hbm, wd_buf, w_sem.at[6], 32)

    def tail(u, carry):
        slot = u % NSLOT
        wait_all(kv_buf.at[slot], kv_sem.at[slot])
        compute_unit(u, slot)
        return carry

    lax.fori_loop(NU - NSLOT + 1, NU, tail, 0)

    hres = x + attn_ref[...]
    xn2 = _layernorm(hres)
    xn2_b = xn2.astype(BF16)
    wait_all(wr_buf, w_sem.at[2])
    wr = wr_buf[...].astype(F32).reshape(1, D)
    r = jnp.sum(xn2_b.astype(F32) * wr, axis=-1, keepdims=True)
    wait_all(wg_buf, w_sem.at[4])
    g = jnp.dot(xn2_b, wg_buf[...], preferred_element_type=F32)
    g = g * jax.nn.sigmoid(g)
    wait_all(wu_buf, w_sem.at[5])
    up = jnp.dot(xn2_b, wu_buf[...], preferred_element_type=F32)
    gu = (g * up).astype(BF16)
    wait_all(wd_buf, w_sem.at[6])
    y = jnp.dot(gu, wd_buf[...], preferred_element_type=F32)
    y = y * jax.nn.sigmoid(r)
    out = hres + (xn2 + (xn2 * 0.0 + y))
    o_ref[...] = out[:B].astype(o_ref.dtype)


@jax.jit
def pallas_sequential_preLN__mha_block_cached__moe_arch_mod__decode_kernel(
    A_x: jax.Array,
    A_k_cache: jax.Array,
    A_v_cache: jax.Array,
    A_wq: jax.Array,
    A_wo: jax.Array,
    B_x: jax.Array,
    B_w_r: jax.Array,
    B_w_gate: jax.Array,
    B_w_up: jax.Array,
    B_w_down: jax.Array,
):
    del B_x
    B, Sq, D = A_x.shape
    _, H, S, Dh = A_k_cache.shape
    F = B_w_gate.shape[1]
    assert Sq == 1

    hbm = pl.BlockSpec(memory_space=pltpu.HBM)
    out = pl.pallas_call(
        functools.partial(_kernel, B=B, H=H, Dh=Dh, S=S, D=D, F=F),
        out_shape=jax.ShapeDtypeStruct((B, D), A_x.dtype),
        in_specs=[hbm] * 9,
        out_specs=pl.BlockSpec(memory_space=pltpu.VMEM),
        scratch_shapes=[
            pltpu.VMEM((NSLOT, 2, B * Dh, BLK), BF16),
            pltpu.VMEM((B, D), BF16),
            pltpu.VMEM((D, H * Dh), BF16),
            pltpu.VMEM((H * Dh, D), BF16),
            pltpu.VMEM((D,), BF16),
            pltpu.VMEM((D, F), BF16),
            pltpu.VMEM((D, F), BF16),
            pltpu.VMEM((F, D), BF16),
            pltpu.VMEM((H, ROWS, Dh), F32),
            pltpu.VMEM((ROWS, B * Dh), F32),
            pltpu.VMEM((ROWS, 1), F32),
            pltpu.VMEM((ROWS, 1), F32),
            pltpu.VMEM((ROWS, B * Dh), F32),
            pltpu.VMEM((ROWS, D), F32),
            pltpu.SemaphoreType.DMA((NSLOT,)),
            pltpu.SemaphoreType.DMA((7,)),
        ],
        compiler_params=pltpu.CompilerParams(
            vmem_limit_bytes=100 * 1024 * 1024,
        ),
    )(
        A_x.reshape(B, D),
        jnp.transpose(A_k_cache, (0, 1, 3, 2)),
        jnp.transpose(A_v_cache, (0, 1, 3, 2)),
        A_wq, A_wo, B_w_r, B_w_gate, B_w_up, B_w_down,
    )
    return out.reshape(B, Sq, D)
```

```python
import jax
import jax.numpy as jnp
from jax import lax
import jax.experimental.pallas as pl
import jax.experimental.pallas.tpu as pltpu

F32 = jnp.float32
BF16 = jnp.bfloat16

ROWS = 8
BLK = 1024
CH_R = 16
NSLOT = 3
NSTREAM = 8
STREAMS = ((0, 0), (1, 1), (2, 0), (3, 1), (0, 1), (1, 0), (2, 1), (3, 0))
NT = (((1,), (1,)), ((), ()))


def _layernorm(x):
    m = jnp.mean(x, axis=-1, keepdims=True)
    xc = x - m
    v = jnp.mean(xc * xc, axis=-1, keepdims=True)
    return xc / jnp.sqrt(v + 1e-5)


def _tiled_copies(src, dst, sem, rows, cols):
    assert src.shape[0] % rows == 0 and src.shape[1] % cols == 0
    tiles = [(pl.ds(i * rows, rows), pl.ds(k * cols, cols))
             for i in range(src.shape[0] // rows)
             for k in range(src.shape[1] // cols)]
    per = len(tiles) // NSTREAM
    assert per * NSTREAM == len(tiles)
    return [pltpu.make_async_copy(src.at[tiles[s * per + t]],
                                  dst.at[tiles[s * per + t]], sem)
            for t in range(per) for s in range(NSTREAM)]


def _start(copies):
    for n, cp in enumerate(copies):
        cp.start(priority=n % 2)


def _wait_filled(dst, sem):
    pltpu.make_async_copy(dst, dst, sem).wait()


def _kernel(x_hbm, k_hbm, v_hbm, wq_hbm, wo_hbm, wr_hbm, wg_hbm, wu_hbm, wd_hbm,
            o_ref,
            kv_buf, x_buf, wq_buf, wo_buf, wr_buf, wg_buf, wu_buf, wd_buf,
            q_buf, m_ref, l_ref, acc_ref, attn_ref, kv_sem, w_sem):
    B, H, Dh, S = k_hbm.shape
    D, F = wg_hbm.shape
    J = S // BLK
    NU = H * J
    scale = Dh ** -0.5
    x_sem, wr_sem, wq_sem, wo_sem, wg_sem, wu_sem, wd_sem = (
        w_sem.at[i] for i in range(7))

    def start_unit(u, slot):
        h = u // J
        keys = pl.ds(pl.multiple_of((u % J) * BLK, BLK), BLK)
        _start([
            pltpu.make_async_copy(
                (k_hbm, v_hbm)[kv].at[b, h, pl.ds(g * CH_R, CH_R), keys],
                kv_buf.at[slot, kv, pl.ds(b * Dh + g * CH_R, CH_R)],
                kv_sem.at[slot])
            for g in range(Dh // CH_R) for b, kv in STREAMS])

    x_cp = pltpu.make_async_copy(x_hbm, x_buf, x_sem)
    wr_cp = pltpu.make_async_copy(wr_hbm, wr_buf, wr_sem)
    x_cp.start()
    _start(_tiled_copies(wq_hbm, wq_buf, wq_sem, 16, 1024))
    wr_cp.start()
    for u in range(NSLOT - 1):
        start_unit(u, u)
    _start(_tiled_copies(wo_hbm, wo_buf, wo_sem, 32, D))

    x_cp.wait()
    x = jnp.concatenate(
        [x_buf[...].astype(F32), jnp.zeros((ROWS - B, D), F32)], axis=0)
    xn = _layernorm(x).astype(BF16)
    _wait_filled(wq_buf, wq_sem)
    q = jnp.dot(xn, wq_buf[...], preferred_element_type=F32)
    for h in range(H):
        q_buf[h] = q[:, h * Dh:(h + 1) * Dh]
    attn_ref[...] = jnp.zeros_like(attn_ref)

    row_s = lax.broadcasted_iota(jnp.int32, (ROWS, BLK), 0)
    row_o = lax.broadcasted_iota(jnp.int32, (ROWS, Dh), 0)

    def compute_unit(u, slot):
        h = u // J
        j = u % J

        @pl.when(j == 0)
        def _():
            m_ref[...] = jnp.full_like(m_ref, -jnp.inf)
            l_ref[...] = jnp.zeros_like(l_ref)
            acc_ref[...] = jnp.zeros_like(acc_ref)

        qh = q_buf[h].astype(BF16)
        s = jnp.zeros((ROWS, BLK), F32)
        for b in range(B):
            sb = jnp.dot(qh, kv_buf[slot, 0, b * Dh:(b + 1) * Dh, :],
                         preferred_element_type=F32)
            s = jnp.where(row_s == b, sb, s)
        s = s * scale
        m_old = m_ref[...]
        m_new = jnp.maximum(m_old, jnp.max(s, axis=-1, keepdims=True))
        m_sub = jnp.where(m_new == -jnp.inf, 0.0, m_new)
        alpha = jnp.exp(m_old - m_sub)
        p = jnp.exp(s - m_sub)
        l_ref[...] = alpha * l_ref[...] + jnp.sum(p, axis=-1, keepdims=True)
        m_ref[...] = m_new
        pv = lax.dot_general(p.astype(BF16), kv_buf[slot, 1], NT,
                             preferred_element_type=F32)
        acc_ref[...] = alpha * acc_ref[...] + pv

        @pl.when(j == J - 1)
        def _():
            @pl.when(h == 0)
            def _():
                _wait_filled(wo_buf, wo_sem)

            acc = acc_ref[...]
            o = jnp.zeros((ROWS, Dh), F32)
            for b in range(B):
                o = jnp.where(row_o == b, acc[:, b * Dh:(b + 1) * Dh], o)
            o = (o / l_ref[...]).astype(BF16)
            wo_h = wo_buf[pl.ds(pl.multiple_of(h * Dh, Dh), Dh), :]
            attn_ref[...] += jnp.dot(o, wo_h, preferred_element_type=F32)

    def body(u, carry):
        slot = u % NSLOT
        _wait_filled(kv_buf.at[slot], kv_sem.at[slot])
        nxt = u + NSLOT - 1
        start_unit(nxt, nxt % NSLOT)
        compute_unit(u, slot)
        return carry

    lax.fori_loop(0, NU - NSLOT + 1, body, 0)

    ffn = (_tiled_copies(wg_hbm, wg_buf, wg_sem, 8, F)
           + _tiled_copies(wu_hbm, wu_buf, wu_sem, 8, F)
           + _tiled_copies(wd_hbm, wd_buf, wd_sem, 32, D))
    per = len(ffn) // (NSLOT - 1)
    assert per * (NSLOT - 1) == len(ffn)
    for t, u in enumerate(range(NU - NSLOT + 1, NU)):
        slot = u % NSLOT
        _wait_filled(kv_buf.at[slot], kv_sem.at[slot])
        _start(ffn[t * per:(t + 1) * per])
        compute_unit(u, slot)

    hres = x + attn_ref[...]
    xn2 = _layernorm(hres)
    xn2_b = xn2.astype(BF16)
    wr_cp.wait()
    wr = wr_buf[...].astype(F32).reshape(1, D)
    r = jnp.sum(xn2_b.astype(F32) * wr, axis=-1, keepdims=True)
    r_sel = jax.nn.sigmoid(r)
    _wait_filled(wg_buf, wg_sem)
    g = jnp.dot(xn2_b, wg_buf[...], preferred_element_type=F32)
    g = g * jax.nn.sigmoid(g)
    _wait_filled(wu_buf, wu_sem)
    up = jnp.dot(xn2_b, wu_buf[...], preferred_element_type=F32)
    gu = (g * up).astype(BF16)
    _wait_filled(wd_buf, wd_sem)
    y = jnp.dot(gu, wd_buf[...], preferred_element_type=F32) * r_sel
    out = hres + (xn2 + (xn2 * 0.0 + y))
    o_ref[...] = out[:B].astype(o_ref.dtype)


@jax.jit
def pallas_sequential_preLN__mha_block_cached__moe_arch_mod__decode_kernel(
    A_x: jax.Array,
    A_k_cache: jax.Array,
    A_v_cache: jax.Array,
    A_wq: jax.Array,
    A_wo: jax.Array,
    B_x: jax.Array,
    B_w_r: jax.Array,
    B_w_gate: jax.Array,
    B_w_up: jax.Array,
    B_w_down: jax.Array,
):
    del B_x
    B, Sq, D = A_x.shape
    _, H, S, Dh = A_k_cache.shape
    F = B_w_gate.shape[1]
    assert Sq == 1 and 2 * B == len(STREAMS)
    assert S % BLK == 0 and Dh % CH_R == 0

    out = pl.pallas_call(
        _kernel,
        out_shape=jax.ShapeDtypeStruct((B, D), A_x.dtype),
        in_specs=[pl.BlockSpec(memory_space=pltpu.HBM)] * 9,
        out_specs=pl.BlockSpec(memory_space=pltpu.VMEM),
        scratch_shapes=[
            pltpu.VMEM((NSLOT, 2, B * Dh, BLK), BF16),
            pltpu.VMEM((B, D), BF16),
            pltpu.VMEM((D, H * Dh), BF16),
            pltpu.VMEM((H * Dh, D), BF16),
            pltpu.VMEM((D,), BF16),
            pltpu.VMEM((D, F), BF16),
            pltpu.VMEM((D, F), BF16),
            pltpu.VMEM((F, D), BF16),
            pltpu.VMEM((H, ROWS, Dh), F32),
            pltpu.VMEM((ROWS, 1), F32),
            pltpu.VMEM((ROWS, 1), F32),
            pltpu.VMEM((ROWS, B * Dh), F32),
            pltpu.VMEM((ROWS, D), F32),
            pltpu.SemaphoreType.DMA((NSLOT,)),
            pltpu.SemaphoreType.DMA((7,)),
        ],
        compiler_params=pltpu.CompilerParams(
            vmem_limit_bytes=64 * 1024 * 1024,
        ),
    )(
        A_x.reshape(B, D),
        jnp.transpose(A_k_cache, (0, 1, 3, 2)),
        jnp.transpose(A_v_cache, (0, 1, 3, 2)),
        A_wq, A_wo, B_w_r, B_w_gate, B_w_up, B_w_down,
    )
    return out.reshape(B, Sq, D)
```
